```python
import os as _os
_os.environ.setdefault("JAX_PLATFORMS", "cpu")
import jax
import jax.numpy as jnp

def _softmax(x, axis=-1):
    return jax.nn.softmax(x, axis=axis)
def _gelu(x):
    return jax.nn.gelu(x, approximate=True)
def _silu(x):
    return jax.nn.silu(x)
def _sigmoid(x):
    return jax.nn.sigmoid(x)
def _layernorm(x, axis=-1, eps=1e-5):
    m = jnp.mean(x, axis=axis, keepdims=True)
    v = jnp.var(x, axis=axis, keepdims=True)
    return (x - m) / jnp.sqrt(v + eps)
def _scatter_add(tgt, idx, src, axis=0):
    return tgt.at[idx].add(src)
def _segment_sum(src, seg, n):
    return jax.ops.segment_sum(src, seg, n)
class _Rng:
    def __init__(self, key):
        self._k = key
    def _next(self):
        self._k, sub = jax.random.split(self._k)
        return sub
    def normal(self, shape):
        return jax.random.normal(self._next(), shape, dtype=jnp.bfloat16)
    def randint(self, lo, hi, shape):
        return jax.random.randint(self._next(), shape, lo, hi, dtype=jnp.int32)
    def uniform(self, shape, lo=0.0, hi=1.0):
        return jax.random.uniform(self._next(), shape, jnp.bfloat16, lo, hi)
    def permutation(self, n):
        return jax.random.permutation(self._next(), n)


kernel_name = 'sequential_preLN__softmax_full_mha__dense_activation_gelu__prompt'

def setup_inputs():
    _rng = _Rng(jax.random.key(int.from_bytes(__import__("os").urandom(4), "little")))
    _w = (lambda a: (lambda t: t.astype(jnp.bfloat16) if jnp.issubdtype(t.dtype, jnp.floating) else t)(jnp.asarray(a)))
    def _A_setup():
        B, S, D = 1, 2048, 640
        return {
            "x": _w((lambda *s: _rng.normal(s) * 0.05)(B, S, D)),
            "wqkv": _w((lambda *s: _rng.normal(s) * 0.05)(D, 3 * D)),
            "wo": _w((lambda *s: _rng.normal(s) * 0.05)(D, D)),
        }
    _A_in = _A_setup()

    def _B_setup():
        B, S, D, F = 1, 2048, 640, 1536
        return {
            "x": _w((lambda *s: _rng.normal(s) * 0.05)(B, S, D)),
            "w1": _w((lambda *s: _rng.normal(s) * 0.4)(D, F) * (D ** -0.5)),
            "b1": _w((lambda *s: _rng.normal(s) * 0.4)(F) * 0.01),
            "w2": _w((lambda *s: _rng.normal(s) * 0.4)(F, D) * (F ** -0.5)),
            "b2": _w((lambda *s: _rng.normal(s) * 0.05)(D) * 0.01),
        }
    _B_in = _B_setup()

    return {
        "A_x": _A_in["x"],
        "A_wqkv": _A_in["wqkv"],
        "A_wo": _A_in["wo"],
        "B_x": _B_in["x"],
        "B_w1": _B_in["w1"],
        "B_b1": _B_in["b1"],
        "B_w2": _B_in["w2"],
        "B_b2": _B_in["b2"],
    }

def reference(A_x, A_wqkv, A_wo, B_x, B_w1, B_b1, B_w2, B_b2):
    def _A_ref(x, wqkv, wo):
        B, S, D = x.shape
        H = 32; Dh = D // H
        qkv = (lambda x, *d: x.transpose(*d))((x @ wqkv).reshape(B, S, 3, H, Dh), 2, 0, 3, 1, 4)
        q, k, v = qkv[0], qkv[1], qkv[2]
        scale = Dh ** -0.5
        scores = jnp.einsum("bhqd,bhkd->bhqk", q, k) * scale
        p = _softmax(scores, axis=-1)
        o = jnp.einsum("bhqk,bhkd->bhqd", p, v)
        return (lambda x, *d: x.transpose(*d))(o, 0, 2, 1, 3).reshape(B, S, D) @ wo

    def _B_ref(x, w1, b1, w2, b2):
        h = jnp.einsum("bsd,df->bsf", x, w1) + b1
        h = _gelu(h)
        return jnp.einsum("bsf,fd->bsd", h, w2) + b2

    x = A_x
    h = x + _A_ref(_layernorm(x, axis=-1), A_wqkv, A_wo)
    h2 = h + _B_ref(_layernorm(h, axis=-1), B_w1, B_b1, B_w2, B_b2)
    return h2
```

```python
import math

import jax
import jax.numpy as jnp
from jax import lax
import jax.experimental.pallas as pl
import jax.experimental.pallas.tpu as pltpu

F32 = jnp.float32
BF16 = jnp.bfloat16
S, D, H, DH, F = 2048, 640, 32, 20, 1536
BQ = 512
NQ = S // BQ
NI = NQ * H
NW = 6
CQ, CE = 64, 16
EPS = 1e-5
QSCALE = DH ** -0.5 * math.log2(math.e)
NT = (((1,), (1,)), ((), ()))


def _dot(a, b):
    return jnp.dot(a, b, preferred_element_type=F32)


def _layernorm(x):
    m = jnp.mean(x, axis=-1, keepdims=True)
    xc = x - m
    v = jnp.mean(xc * xc, axis=-1, keepdims=True)
    return xc * lax.rsqrt(v + EPS)


def _gelu(x):
    c = math.sqrt(2.0 / math.pi)
    u = x * (c + (c * 0.044715) * (x * x))
    hx = 0.5 * x
    return hx + hx * jnp.tanh(u)


def _kernel(x_hbm, wqkv_hbm, wo_hbm, w1_hbm, b1_ref, w2_hbm, b2_ref, out_hbm,
            x_v, wqkv_v, wo_v, w1_v, w2_v, out_v, wk_v, wqt_v, wvt_v,
            kw, qt, vt, ot, s0, s1, p0, p1, m0, m1, sems, osems):
    def rows(ref, j):
        return ref.at[pl.ds(pl.multiple_of(j * BQ, BQ), BQ)]

    def x_copy(j):
        return pltpu.make_async_copy(rows(x_hbm, j), rows(x_v, j), sems.at[4 + j])

    def out_copy(j):
        return pltpu.make_async_copy(rows(out_v, j), rows(out_hbm, j), osems.at[j])

    w_copies = [pltpu.make_async_copy(a, b, sems.at[n]) for n, (a, b) in enumerate(
        ((wqkv_hbm, wqkv_v), (wo_hbm, wo_v), (w1_hbm, w1_v), (w2_hbm, w2_v)))]
    w_copies[0].start()
    for j in range(NQ):
        x_copy(j).start()
    for c in w_copies[1:]:
        c.start()

    ot[...] = jnp.zeros(ot.shape, F32)
    w_copies[0].wait()
    wqt_v[...] = wqkv_v[:, 0:D].T
    wvt_v[...] = wqkv_v[:, 2 * D:3 * D].T
    for g in range(NW):
        st = D + min(6 * DH * g, D - 128)
        wk_v[:, g * 128:(g + 1) * 128] = wqkv_v[:, st:st + 128]

    def proj(j, carry):
        r0 = pl.multiple_of(j * BQ, BQ)
        x_copy(j).wait()
        xn = _layernorm(x_v[pl.ds(r0, BQ), :].astype(F32)).astype(BF16)
        k = _dot(xn, wk_v[...]).astype(BF16)
        for g in range(NW):
            kw[g, pl.ds(r0, BQ), :] = k[:, g * 128:(g + 1) * 128]
        qt[:, pl.ds(r0, BQ)] = lax.dot_general(
            wqt_v[...], xn, NT, preferred_element_type=F32) * QSCALE
        v = lax.dot_general(wvt_v[...], xn, NT, preferred_element_type=F32)
        r = lax.broadcasted_iota(jnp.int32, (32, BQ), 0)
        for h in range(H):
            st = DH * h // 16 * 16
            off = DH * h - st
            vt[h, :, pl.ds(r0, BQ)] = jnp.where(
                (r >= off) & (r < off + DH), v[st:st + 32, :], 1.0).astype(BF16)
        return carry

    lax.fori_loop(0, NQ, proj, 0)

    def q_operand(it):
        h = it % H
        q0 = pl.multiple_of((it // H) * BQ, BQ)
        g = h // 6
        st = pl.multiple_of(jnp.minimum(6 * DH * g, D - 128), 8)
        lo = DH * h - st
        r = lax.broadcasted_iota(jnp.int32, (128, BQ), 0)
        q = jnp.where((r >= lo) & (r < lo + DH), qt[pl.ds(st, 128), pl.ds(q0, BQ)], 0.0)
        return g, q.astype(BF16)

    def qk_exp(it, s_out, m_out, s_in, m_in, p_out):
        if s_out is not None:
            g, q = q_operand(it)
        if s_in is not None:
            m = jnp.broadcast_to(jnp.max(m_in[...], axis=0, keepdims=True), (CE, BQ))
        mx = None
        for c in range(S // CQ):
            if s_out is not None:
                s = _dot(kw[g, c * CQ:(c + 1) * CQ, :], q)
                s_out[c * CQ:(c + 1) * CQ, :] = s
                t = jnp.max(s.reshape(CQ // 8, 8, BQ), axis=0)
                mx = t if mx is None else jnp.maximum(mx, t)
            if s_in is not None:
                for e in range(CQ // CE):
                    a = c * CQ + e * CE
                    p_out[a:a + CE, :] = jnp.exp2(s_in[a:a + CE, :] - m).astype(BF16)
        if s_out is not None:
            m_out[...] = mx

    def pv(it, p_in):
        h = it % H
        acc = _dot(vt[h], p_in[...])
        st = pl.multiple_of(DH * h // 16 * 16, 16)
        off = DH * h - st
        l = jnp.where(off == 0, acc[31:32], acc[0:1])
        r = lax.broadcasted_iota(jnp.int32, (32, BQ), 0)
        ot[pl.ds(st, 32), :] = jnp.where(
            (r >= off) & (r < off + DH), acc * (1.0 / l), ot[pl.ds(st, 32), :])

    def tail(j):
        r0 = pl.multiple_of(j * BQ, BQ)
        o = ot[...].T.astype(BF16)
        h = x_v[pl.ds(r0, BQ), :].astype(F32) + _dot(o, wo_v[...])
        hn = _layernorm(h).astype(BF16)
        a = _gelu(_dot(hn, w1_v[...]) + b1_ref[...].astype(F32)).astype(BF16)
        y = h + (_dot(a, w2_v[...]) + b2_ref[...].astype(F32))
        out_v[pl.ds(r0, BQ), :] = y.astype(BF16)
        out_copy(j).start()

    qk_exp(0, s0, m0, None, None, None)
    qk_exp(1, s1, m1, s0, m0, p0)
    for c in w_copies[1:]:
        c.wait()

    def step(i, carry):
        nxt = jnp.minimum(i + 2, NI - 1)

        @pl.when(i % 2 == 0)
        def _():
            qk_exp(nxt, s0, m0, s1, m1, p1)
            pv(i, p0)

        @pl.when(i % 2 == 1)
        def _():
            qk_exp(nxt, s1, m1, s0, m0, p0)
            pv(i, p1)

        @pl.when(i % H == H - 1)
        def _():
            tail(i // H)

        return carry

    lax.fori_loop(0, NI, step, 0)
    for j in range(NQ):
        out_copy(j).wait()


@jax.jit
def pallas_sequential_preLN__softmax_full_mha__dense_activation_gelu__prompt_kernel(
    A_x: jax.Array,
    A_wqkv: jax.Array,
    A_wo: jax.Array,
    B_x: jax.Array,
    B_w1: jax.Array,
    B_b1: jax.Array,
    B_w2: jax.Array,
    B_b2: jax.Array,
):
    del B_x
    hbm = pl.BlockSpec(memory_space=pl.ANY)
    vmem = pl.BlockSpec(memory_space=pltpu.VMEM)
    out = pl.pallas_call(
        _kernel,
        in_specs=[hbm, hbm, hbm, hbm, vmem, hbm, vmem],
        out_specs=hbm,
        out_shape=jax.ShapeDtypeStruct((S, D), BF16),
        scratch_shapes=[
            pltpu.VMEM((S, D), BF16),
            pltpu.VMEM((D, 3 * D), BF16),
            pltpu.VMEM((D, D), BF16),
            pltpu.VMEM((D, F), BF16),
            pltpu.VMEM((F, D), BF16),
            pltpu.VMEM((S, D), BF16),
            pltpu.VMEM((D, NW * 128), BF16),
            pltpu.VMEM((D, D), BF16),
            pltpu.VMEM((D, D), BF16),
            pltpu.VMEM((NW, S, 128), BF16),
            pltpu.VMEM((D, S), F32),
            pltpu.VMEM((H, 32, S), BF16),
            pltpu.VMEM((D, BQ), F32),
            pltpu.VMEM((S, BQ), F32),
            pltpu.VMEM((S, BQ), F32),
            pltpu.VMEM((S, BQ), BF16),
            pltpu.VMEM((S, BQ), BF16),
            pltpu.VMEM((8, BQ), F32),
            pltpu.VMEM((8, BQ), F32),
            pltpu.SemaphoreType.DMA((4 + NQ,)),
            pltpu.SemaphoreType.DMA((NQ,)),
        ],
        compiler_params=pltpu.CompilerParams(vmem_limit_bytes=100 * 2**20),
        name="block",
    )(A_x.reshape(S, D), A_wqkv, A_wo, B_w1, B_b1.reshape(1, F), B_w2, B_b2.reshape(1, D))
    return out.reshape(1, S, D)
```

```python
import math

import jax
import jax.numpy as jnp
from jax import lax
import jax.experimental.pallas as pl
import jax.experimental.pallas.tpu as pltpu

F32 = jnp.float32
BF16 = jnp.bfloat16
S, D, H, DH, F = 2048, 640, 32, 20, 1536
BQ = 512
NQ = S // BQ
NI = NQ * H
NW = 6
CQ, CE = 64, 32
EPS = 1e-5
QSCALE = DH ** -0.5 * math.log2(math.e)
NT = (((1,), (1,)), ((), ()))


def _dot(a, b):
    return jnp.dot(a, b, preferred_element_type=F32)


def _layernorm(x):
    m = jnp.mean(x, axis=-1, keepdims=True)
    xc = x - m
    v = jnp.mean(xc * xc, axis=-1, keepdims=True)
    return xc * lax.rsqrt(v + EPS)


def _gelu(x):
    c = math.sqrt(2.0 / math.pi)
    u = x * (c + (c * 0.044715) * (x * x))
    hx = 0.5 * x
    return hx + hx * jnp.tanh(u)


def _kernel(x_hbm, wqkv_hbm, wo_hbm, w1_hbm, b1_ref, w2_hbm, b2_ref, out_hbm,
            x_v, wqkv_v, wo_v, w1_v, w2_v, out_v, wk_v, wqt_v, wvt_v,
            kw, qt, vt, ot, oh, qb, s0, s1, p0, p1, m0, m1, sems, osems):
    def rows(ref, j):
        return ref.at[pl.ds(pl.multiple_of(j * BQ, BQ), BQ)]

    def x_copy(j):
        return pltpu.make_async_copy(rows(x_hbm, j), rows(x_v, j), sems.at[4 + j])

    def out_copy(j):
        return pltpu.make_async_copy(rows(out_v, j), rows(out_hbm, j), osems.at[j])

    w_copies = [pltpu.make_async_copy(a, b, sems.at[n]) for n, (a, b) in enumerate(
        ((wqkv_hbm, wqkv_v), (wo_hbm, wo_v), (w1_hbm, w1_v), (w2_hbm, w2_v)))]
    w_copies[0].start()
    for j in range(NQ):
        x_copy(j).start()

    ot[...] = jnp.zeros(ot.shape, F32)
    w_copies[0].wait()
    for c in w_copies[1:]:
        c.start()
    wqt_v[...] = wqkv_v[:, 0:D].T
    wvt_v[...] = wqkv_v[:, 2 * D:3 * D].T
    for g in range(NW):
        st = D + min(6 * DH * g, D - 128)
        wk_v[:, g * 128:(g + 1) * 128] = wqkv_v[:, st:st + 128]

    def proj(j, carry):
        r0 = pl.multiple_of(j * BQ, BQ)
        x_copy(j).wait()
        xn = _layernorm(x_v[pl.ds(r0, BQ), :].astype(F32)).astype(BF16)
        k = _dot(xn, wk_v[...]).astype(BF16)
        for g in range(NW):
            kw[g, pl.ds(r0, BQ), :] = k[:, g * 128:(g + 1) * 128]
        qt[:, pl.ds(r0, BQ)] = lax.dot_general(
            wqt_v[...], xn, NT, preferred_element_type=F32) * QSCALE
        v = lax.dot_general(wvt_v[...], xn, NT, preferred_element_type=F32)
        r = lax.broadcasted_iota(jnp.int32, (32, BQ), 0)
        for h in range(H):
            st = DH * h // 16 * 16
            off = DH * h - st
            vt[h, :, pl.ds(r0, BQ)] = jnp.where(
                (r >= off) & (r < off + DH), v[st:st + 32, :], 1.0).astype(BF16)
        return carry

    lax.fori_loop(0, NQ, proj, 0)

    def q_operand(it):
        h = it % H
        q0 = pl.multiple_of((it // H) * BQ, BQ)
        g = h // 6
        st = pl.multiple_of(jnp.minimum(6 * DH * g, D - 128), 8)
        lo = DH * h - st
        r = lax.broadcasted_iota(jnp.int32, (128, BQ), 0)
        q = jnp.where((r >= lo) & (r < lo + DH), qt[pl.ds(st, 128), pl.ds(q0, BQ)], 0.0)
        return g, q.astype(BF16)

    def qk_exp(it, s_out, m_out, s_in, m_in, p_out):
        if s_out is not None:
            g, q = (it % H) // 6, qb[...]
            qb[...] = q_operand(jnp.minimum(it + 1, NI - 1))[1]
        if s_in is not None:
            m = jnp.broadcast_to(jnp.max(m_in[...], axis=0, keepdims=True), (CE, BQ))
        mx = None
        for c in range(S // CQ):
            if s_out is not None:
                s = _dot(kw[g, c * CQ:(c + 1) * CQ, :], q)
                s_out[c * CQ:(c + 1) * CQ, :] = s
                t = jnp.max(s.reshape(CQ // 8, 8, BQ), axis=0)
                mx = t if mx is None else jnp.maximum(mx, t)
            if s_in is not None:
                for e in range(CQ // CE):
                    a = c * CQ + e * CE
                    p_out[a:a + CE, :] = jnp.exp2(s_in[a:a + CE, :] - m).astype(BF16)
        if s_out is not None:
            m_out[...] = mx

    def pv(it, p_in):
        h = it % H
        oh[h] = _dot(vt[h], p_in[...])

    def tail(j):
        r0 = pl.multiple_of(j * BQ, BQ)
        r = lax.broadcasted_iota(jnp.int32, (32, BQ), 0)
        for h in range(H):
            st = DH * h // 16 * 16
            off = DH * h - st
            acc = oh[h]
            l = acc[31:32] if off == 0 else acc[0:1]
            ot[st:st + 32, :] = jnp.where(
                (r >= off) & (r < off + DH), acc * (1.0 / l), ot[st:st + 32, :])
        o = ot[...].T.astype(BF16)
        h = x_v[pl.ds(r0, BQ), :].astype(F32) + _dot(o, wo_v[...])
        hn = _layernorm(h).astype(BF16)
        a = _gelu(_dot(hn, w1_v[...]) + b1_ref[...].astype(F32).reshape(1, F)).astype(BF16)
        y = h + (_dot(a, w2_v[...]) + b2_ref[...].astype(F32).reshape(1, D))
        out_v[pl.ds(r0, BQ), :] = y.astype(BF16)
        out_copy(j).start()

    qb[...] = q_operand(0)[1]
    qk_exp(0, s0, m0, None, None, None)
    qk_exp(1, s1, m1, s0, m0, p0)
    for c in w_copies[1:]:
        c.wait()

    def step(i, carry):
        nxt = i + 2

        @pl.when(i == NI - 2)
        def _():
            pv(i, p0)
            qk_exp(nxt, None, None, s1, m1, p1)

        @pl.when(i == NI - 1)
        def _():
            pv(i, p1)

        @pl.when((i % 2 == 0) & (i < NI - 2))
        def _():
            qk_exp(nxt, s0, m0, s1, m1, p1)
            pv(i, p0)

        @pl.when((i % 2 == 1) & (i < NI - 2))
        def _():
            qk_exp(nxt, s1, m1, s0, m0, p0)
            pv(i, p1)

        @pl.when(i % H == H - 1)
        def _():
            tail(i // H)

        return carry

    lax.fori_loop(0, NI, step, 0)
    for j in range(NQ):
        out_copy(j).wait()


@jax.jit
def pallas_sequential_preLN__softmax_full_mha__dense_activation_gelu__prompt_kernel(
    A_x: jax.Array,
    A_wqkv: jax.Array,
    A_wo: jax.Array,
    B_x: jax.Array,
    B_w1: jax.Array,
    B_b1: jax.Array,
    B_w2: jax.Array,
    B_b2: jax.Array,
):
    del B_x
    hbm = pl.BlockSpec(memory_space=pl.ANY)
    vmem = pl.BlockSpec(memory_space=pltpu.VMEM)
    out = pl.pallas_call(
        _kernel,
        in_specs=[hbm, hbm, hbm, hbm, vmem, hbm, vmem],
        out_specs=hbm,
        out_shape=jax.ShapeDtypeStruct((S, D), BF16),
        scratch_shapes=[
            pltpu.VMEM((S, D), BF16),
            pltpu.VMEM((D, 3 * D), BF16),
            pltpu.VMEM((D, D), BF16),
            pltpu.VMEM((D, F), BF16),
            pltpu.VMEM((F, D), BF16),
            pltpu.VMEM((S, D), BF16),
            pltpu.VMEM((D, NW * 128), BF16),
            pltpu.VMEM((D, D), BF16),
            pltpu.VMEM((D, D), BF16),
            pltpu.VMEM((NW, S, 128), BF16),
            pltpu.VMEM((D, S), F32),
            pltpu.VMEM((H, 32, S), BF16),
            pltpu.VMEM((D, BQ), F32),
            pltpu.VMEM((H, 32, BQ), F32),
            pltpu.VMEM((128, BQ), BF16),
            pltpu.VMEM((S, BQ), F32),
            pltpu.VMEM((S, BQ), F32),
            pltpu.VMEM((S, BQ), BF16),
            pltpu.VMEM((S, BQ), BF16),
            pltpu.VMEM((8, BQ), F32),
            pltpu.VMEM((8, BQ), F32),
            pltpu.SemaphoreType.DMA((4 + NQ,)),
            pltpu.SemaphoreType.DMA((NQ,)),
        ],
        compiler_params=pltpu.CompilerParams(vmem_limit_bytes=100 * 2**20),
        name="block",
    )(A_x.reshape(S, D), A_wqkv, A_wo, B_w1, B_b1, B_w2, B_b2)
    return out.reshape(1, S, D)
```
